```python
import os as _os
_os.environ.setdefault("JAX_PLATFORMS", "cpu")
import jax
import jax.numpy as jnp

def _softmax(x, axis=-1):
    return jax.nn.softmax(x, axis=axis)
def _gelu(x):
    return jax.nn.gelu(x, approximate=True)
def _silu(x):
    return jax.nn.silu(x)
def _sigmoid(x):
    return jax.nn.sigmoid(x)
def _layernorm(x, axis=-1, eps=1e-5):
    m = jnp.mean(x, axis=axis, keepdims=True)
    v = jnp.var(x, axis=axis, keepdims=True)
    return (x - m) / jnp.sqrt(v + eps)
def _scatter_add(tgt, idx, src, axis=0):
    return tgt.at[idx].add(src)
def _segment_sum(src, seg, n):
    return jax.ops.segment_sum(src, seg, n)
class _Rng:
    def __init__(self, key):
        self._k = key
    def _next(self):
        self._k, sub = jax.random.split(self._k)
        return sub
    def normal(self, shape):
        return jax.random.normal(self._next(), shape, dtype=jnp.bfloat16)
    def randint(self, lo, hi, shape):
        return jax.random.randint(self._next(), shape, lo, hi, dtype=jnp.int32)
    def uniform(self, shape, lo=0.0, hi=1.0):
        return jax.random.uniform(self._next(), shape, jnp.bfloat16, lo, hi)
    def permutation(self, n):
        return jax.random.permutation(self._next(), n)


kernel_name = 'concat_heads__mha_block_cached__mha_block_cached__near_ridge'

def setup_inputs():
    _rng = _Rng(jax.random.key(int.from_bytes(__import__("os").urandom(4), "little")))
    _w = (lambda a: (lambda t: t.astype(jnp.bfloat16) if jnp.issubdtype(t.dtype, jnp.floating) else t)(jnp.asarray(a)))
    def _A_setup():
        B, Sq, D = 16, 32, 1024
        H, Sk, Dh = 32, 32, 128
        return {
            "x": _w((lambda *s: _rng.normal(s) * 0.8)(B, Sq, D)),
            "k_cache": _w((lambda *s: _rng.normal(s) * 0.8)(B, H, Sk, Dh)),
            "v_cache": _w((lambda *s: _rng.normal(s) * 0.05)(B, H, Sk, Dh)),
            "wq": _w((lambda *s: _rng.normal(s) * 0.8)(D, H * Dh) * (D ** -0.5)),
            "wo": _w((lambda *s: _rng.normal(s) * 0.05)(H * Dh, D) * ((H * Dh) ** -0.5)),
        }
    _A_in = _A_setup()

    def _B_setup():
        B, Sq, D = 16, 32, 1024
        H, Sk, Dh = 32, 32, 128
        return {
            "x": _w((lambda *s: _rng.normal(s) * 0.8)(B, Sq, D)),
            "k_cache": _w((lambda *s: _rng.normal(s) * 0.8)(B, H, Sk, Dh)),
            "v_cache": _w((lambda *s: _rng.normal(s) * 0.05)(B, H, Sk, Dh)),
            "wq": _w((lambda *s: _rng.normal(s) * 0.8)(D, H * Dh) * (D ** -0.5)),
            "wo": _w((lambda *s: _rng.normal(s) * 0.05)(H * Dh, D) * ((H * Dh) ** -0.5)),
        }
    _B_in = _B_setup()

    return {
        "A_x": _A_in["x"],
        "A_k_cache": _A_in["k_cache"],
        "A_v_cache": _A_in["v_cache"],
        "A_wq": _A_in["wq"],
        "A_wo": _A_in["wo"],
        "B_x": _B_in["x"],
        "B_k_cache": _B_in["k_cache"],
        "B_v_cache": _B_in["v_cache"],
        "B_wq": _B_in["wq"],
        "B_wo": _B_in["wo"],
    }

def reference(A_x, A_k_cache, A_v_cache, A_wq, A_wo, B_x, B_k_cache, B_v_cache, B_wq, B_wo):
    def _A_ref(x, k_cache, v_cache, wq, wo):
        B, Sq, D = x.shape
        H, Dh = 32, 128
        q = (lambda x, *d: x.transpose(*d))((x @ wq).reshape(B, Sq, H, Dh), 0, 2, 1, 3)
        scores = jnp.einsum("bhqd,bhkd->bhqk", q, k_cache) * (Dh ** -0.5)
        p = _softmax(scores, axis=-1)
        o = jnp.einsum("bhqk,bhkd->bhqd", p, v_cache)
        return (lambda x, *d: x.transpose(*d))(o, 0, 2, 1, 3).reshape(B, Sq, H * Dh) @ wo

    def _B_ref(x, k_cache, v_cache, wq, wo):
        B, Sq, D = x.shape
        H, Dh = 32, 128
        q = (lambda x, *d: x.transpose(*d))((x @ wq).reshape(B, Sq, H, Dh), 0, 2, 1, 3)
        scores = jnp.einsum("bhqd,bhkd->bhqk", q, k_cache) * (Dh ** -0.5)
        p = _softmax(scores, axis=-1)
        o = jnp.einsum("bhqk,bhkd->bhqd", p, v_cache)
        return (lambda x, *d: x.transpose(*d))(o, 0, 2, 1, 3).reshape(B, Sq, H * Dh) @ wo

    a = _A_ref(A_x, A_k_cache, A_v_cache, A_wq, A_wo)
    b = _B_ref(B_x, B_k_cache, B_v_cache, B_wq, B_wo)
    return jnp.concatenate([a, b], axis=-1)
```

```python
import functools

import jax
import jax.numpy as jnp
from jax import lax
import jax.experimental.pallas as pl
import jax.experimental.pallas.tpu as pltpu

B, SQ, D = 16, 32, 1024
H, SK, DH = 32, 32, 128
M = B * SQ
KT = D // DH
GB = 128 // SQ
IH = 16
NI = 4
IW = IH * DH
PRE = 12
PW = PRE * DH
GH = 4
GW = GH * DH
WQ_PAD = 128
TAIL_CHUNKS = 4
EXP_SCALE = DH ** -0.5 * 1.4426950408889634
NT_DIMS = (((1,), (1,)), ((), ()))
F32 = jnp.float32
BF16 = jnp.bfloat16

CUTS = (1, 4, 8, 15, 28, 48)
SEM_XB = len(CUTS)
SEM_S2 = SEM_XB + 1
SEM_S3 = SEM_S2 + 2
SEM_OUT = SEM_S3 + NI
NUM_SEMS = SEM_OUT + 1


def _stage1_plan():
    tiles = [(k, n) for k in range(KT) for n in range(2 * PRE)]
    segs, seen_k, lo = [], 0, 0
    for c in CUTS:
        ts = tiles[lo:4 * c]
        lo = 4 * c
        kr = {}
        for k, n in ts:
            a, b = kr.get(n, (k, k + 1))
            kr[n] = (min(a, k), max(b, k + 1))
        rects = []
        for n in sorted(kr):
            if rects and rects[-1][:2] == kr[n] and rects[-1][3] == n and n != PRE:
                rects[-1] = (*kr[n], rects[-1][2], n + 1)
            else:
                rects.append((*kr[n], n, n + 1))
        k_end = max(seen_k, max(k for k, _ in ts) + 1)
        segs.append(((seen_k, k_end), rects))
        seen_k = k_end
    assert lo == len(tiles)
    return segs


SEGS = _stage1_plan()


def _kernel(xa, ka, va, wqa, woa, xb, kb, vb, wqb, wob, out_hbm,
            x_buf, wq_buf, k_buf, v_buf, wo_buf, q_buf, o_buf, qacc, acc, out_buf, sems, cnt):
    k_hbm, v_hbm, wq_hbm, wo_hbm = (ka, kb), (va, vb), (wqa, wqb), (woa, wob)
    copy = pltpu.make_async_copy

    groups = []
    for (xk0, xk1), rects in SEGS:
        g = []
        for k0, k1, n0, n1 in rects:
            it, c0 = divmod(n0, PRE)
            c0, c1 = c0 * DH, (c0 + n1 - n0) * DH
            g.append((wqa.at[k0 * DH:k1 * DH, it * IW + c0:it * IW + c1],
                      wq_buf.at[it, k0 * DH:k1 * DH, c0:c1]))
        if xk1 > xk0:
            g.append((xa.at[:, xk0 * DH:xk1 * DH], x_buf.at[0, :, xk0 * DH:xk1 * DH]))
        groups.append(g)
    groups.append([(xb, x_buf.at[1])])
    for j in range(2):
        groups.append([(wqb.at[:, j * IW:j * IW + PW], wq_buf.at[2 + j, :, 0:PW])])
    for i in range(NI):
        blk, half = divmod(i, 2)
        groups.append([
            (wq_hbm[blk].at[:, half * IW + PW:(half + 1) * IW], wq_buf.at[i, :, PW:IW]),
            (k_hbm[blk].at[:, half * IH:(half + 1) * IH], k_buf.at[i]),
            (v_hbm[blk].at[:, half * IH:(half + 1) * IH], v_buf.at[i]),
            (wo_hbm[blk].at[half * IW:(half + 1) * IW, :], wo_buf.at[i]),
        ])

    for g, group in enumerate(groups):
        for src, dst in group:
            copy(src, dst, sems.at[g]).start()

    def wait_group(g):
        for src, dst in groups[g]:
            copy(src, dst, sems.at[g]).wait()

    def out_chunks(n):
        rows = M // TAIL_CHUNKS if n == D // DH - 1 else M
        return [(r0, rows) for r0 in range(0, M, rows)]

    def out_copy(blk, n, r0, rows):
        return copy(out_buf.at[blk, r0:r0 + rows, n * DH:(n + 1) * DH],
                    out_hbm.at[r0:r0 + rows, pl.ds(pl.multiple_of(blk * D + n * DH, DH), DH)],
                    sems.at[SEM_OUT])

    def stage1():
        for si, (_, rects) in enumerate(SEGS):
            wait_group(si)
            for k0, k1, n0, n1 in rects:
                it, c0 = divmod(n0, PRE)
                step = (n1 - n0) if k1 - k0 < 4 else 1
                for n in range(n0, n1, step):
                    ca = (c0 + n - n0) * DH
                    cb = ca + step * DH
                    r = jnp.dot(x_buf[0, :, k0 * DH:k1 * DH], wq_buf[it, k0 * DH:k1 * DH, ca:cb],
                                preferred_element_type=F32)
                    if k0 > 0:
                        r = qacc[:, n * DH:(n + step) * DH] + r
                    if k1 < KT:
                        qacc[:, n * DH:(n + step) * DH] = r
                    else:
                        q_buf[it, :, ca:cb] = r.astype(BF16)

    def stage2(j, carry):
        dst = wq_buf.at[2 + j, :, 0:PW]
        copy(dst, dst, sems.at[SEM_S2 + j]).wait()
        for c0 in range(0, PW, DH):
            q = jnp.dot(x_buf[1], wq_buf[2 + j, :, c0:c0 + DH], preferred_element_type=F32)
            q_buf[2 + j, :, c0:c0 + DH] = q.astype(BF16)
        return carry

    def stage3(i, carry):
        for dst in (wq_buf.at[i, :, PW:IW], k_buf.at[i], v_buf.at[i], wo_buf.at[i]):
            copy(dst, dst, sems.at[SEM_S3 + i]).wait()
        blk = lax.shift_right_logical(i, 1)
        second_half = (i & 1) == 1
        row = lax.broadcasted_iota(jnp.int32, (128, 128), 0) // SQ
        col = lax.broadcasted_iota(jnp.int32, (128, 128), 1) // SK
        same_batch = row == col

        def qk_softmax(h):
            ps = []
            for g in range(B // GB):
                qg = q_buf[i, g * 128:(g + 1) * 128, h * DH:(h + 1) * DH]
                kg = k_buf[i, GB * g:GB * (g + 1), h].reshape(128, DH)
                s = lax.dot_general(qg, kg, NT_DIMS, preferred_element_type=F32)
                s = jnp.where(same_batch, s, -jnp.inf)
                m = jnp.max(s, axis=-1, keepdims=True)
                e = jnp.exp2((s - m) * EXP_SCALE)
                l = jnp.sum(e, axis=-1, keepdims=True)
                r = pl.reciprocal(l, approx=True)
                r = r * (2.0 - l * r)
                ps.append((e * r).astype(BF16))
            return ps

        def pv(h, ps):
            for g in range(B // GB):
                vg = v_buf[i, GB * g:GB * (g + 1), h].reshape(128, DH)
                o = jnp.dot(ps[g], vg, preferred_element_type=F32)
                o_buf[g * 128:(g + 1) * 128, h * DH:(h + 1) * DH] = o.astype(BF16)

        q_part = {}

        def q_round(hh, half):
            c = PW + hh * DH
            ks = slice(half * (D // 2), (half + 1) * (D // 2))
            r = jnp.dot(x_buf[blk, :, ks], wq_buf[i, ks, c:c + DH], preferred_element_type=F32)
            if half == 0:
                q_part[hh] = r
            else:
                q_buf[i, :, c:c + DH] = (q_part.pop(hh) + r).astype(BF16)

        def o_round(g, n):
            cs = slice(n * DH, (n + 1) * DH)
            r = jnp.dot(o_buf[:, g * GW:(g + 1) * GW], wo_buf[i, g * GW:(g + 1) * GW, cs],
                        preferred_element_type=F32)
            prev = acc[:, cs]
            if g == 0:
                prev = jnp.where(second_half, prev, 0.0)
            s = prev + r
            acc[:, cs] = s
            if g == IH // GH - 1:
                for r0, rows in out_chunks(n):
                    out_buf[blk, r0:r0 + rows, cs] = s[r0:r0 + rows].astype(BF16)

                    @pl.when(second_half)
                    def _():
                        out_copy(blk, n, r0, rows).start()

        rounds = [functools.partial(q_round, hh, half) for hh in range(IH - PRE) for half in range(2)]
        rounds += [functools.partial(o_round, g, n) for g in range(IH // GH) for n in range(D // DH)]
        ps = {}
        for step, rd in enumerate(rounds):
            rd()
            if 0 <= step - 3 < IH:
                pv(step - 3, ps.pop(step - 3))
            if 0 <= step - 1 < IH:
                ps[step - 1] = qk_softmax(step - 1)
        return carry

    def body(_, carry):
        stage1()
        wait_group(SEM_XB)
        lax.fori_loop(0, 2, stage2, 0)
        lax.fori_loop(0, NI, stage3, 0)
        for blk in range(2):
            for n in range(D // DH):
                for r0, rows in out_chunks(n):
                    out_copy(blk, n, r0, rows).wait()
        return carry

    cnt[0] = 1
    lax.fori_loop(0, cnt[0], body, 0)


@jax.jit
def pallas_concat_heads__mha_block_cached__mha_block_cached__near_ridge_kernel(
    A_x: jax.Array,
    A_k_cache: jax.Array,
    A_v_cache: jax.Array,
    A_wq: jax.Array,
    A_wo: jax.Array,
    B_x: jax.Array,
    B_k_cache: jax.Array,
    B_v_cache: jax.Array,
    B_wq: jax.Array,
    B_wo: jax.Array,
):
    out = pl.pallas_call(
        _kernel,
        in_specs=[pl.BlockSpec(memory_space=pl.ANY)] * 10,
        out_specs=pl.BlockSpec(memory_space=pl.ANY),
        out_shape=jax.ShapeDtypeStruct((M, 2 * D), BF16),
        scratch_shapes=[
            pltpu.VMEM((2, M, D), BF16),
            pltpu.VMEM((NI, D, IW + WQ_PAD), BF16),
            pltpu.VMEM((NI, B, IH, SK, DH), BF16),
            pltpu.VMEM((NI, B, IH, SK, DH), BF16),
            pltpu.VMEM((NI, IW, D), BF16),
            pltpu.VMEM((NI, M, IW), BF16),
            pltpu.VMEM((M, IW), BF16),
            pltpu.VMEM((M, 2 * PW), F32),
            pltpu.VMEM((M, D), F32),
            pltpu.VMEM((2, M, D), BF16),
            pltpu.SemaphoreType.DMA((NUM_SEMS,)),
            pltpu.SMEM((1,), jnp.int32),
        ],
        compiler_params=pltpu.CompilerParams(
            vmem_limit_bytes=100 * 1024 * 1024,
            disable_bounds_checks=True,
            disable_semaphore_checks=True,
        ),
    )(A_x.reshape(M, D), A_k_cache, A_v_cache, A_wq, A_wo,
      B_x.reshape(M, D), B_k_cache, B_v_cache, B_wq, B_wo)
    return out.reshape(B, SQ, 2 * D)
```

```python
import functools

import jax
import jax.numpy as jnp
from jax import lax
import jax.experimental.pallas as pl
import jax.experimental.pallas.tpu as pltpu

B, SQ, D = 16, 32, 1024
H, SK, DH = 32, 32, 128
M = B * SQ
KT = D // DH
GB = 128 // SQ
IH = 16
NI = 4
IW = IH * DH
PRE = 12
PW = PRE * DH
GH = 4
GW = GH * DH
W_PAD = 128
TAIL_CHUNKS = 4
P16 = 20
P32 = 36
EXP_SCALE = DH ** -0.5 * 1.4426950408889634
NT_DIMS = (((1,), (1,)), ((), ()))
F32 = jnp.float32
BF16 = jnp.bfloat16
U32 = jnp.uint32

UH, XH, WH = 8, 2, 4
X0 = UH
M0 = UH + XH
W0 = IH - WH
MHEADS = range(M0, W0)
AS = 8

CUTS = (1, 4, 8, 15, 28, 48)

GORDER = (2, 0, 1, 3)
QK_AT = (0, 1)
PV_AT = (14, 14, 14, 14, 16, 17, 18, 19, 0, 0, 2, 3, 27, 28, 29, 30)
PREP3 = (1800, 2500, 3500, 5200, 5200, 6600, 5500, 7500, 10500, 13064, 7436, 9000, 14100, 17000)
SPAN3 = (0, 22270)
PROF3 = ((0, 1.0),)
PREP2 = (0, 512, 512, 1400, 500, 500, 7000, 9000, 500, 1200, 1800, 3600, 2400, 4400)
SPAN2 = (1700, 11850)
PROF2 = ((0, 1.0), (5000, 1.03), (9300, 1.0))
DBLK = 2
SMB = 2
SMC = 16
SMC2 = 16
CPB = 4
CPB2 = 2
LAG = 900
CAP = 3.3
LC = (96, 64, 140, 400, 500, 40, 8)

SEM_XB = len(CUTS)
SEM_S2 = SEM_XB + 1
SEM_S3 = SEM_S2 + 2
SEM_KU = SEM_S3 + NI
SEM_OUT = SEM_KU + NI - 1
NUM_SEMS = SEM_OUT + 1


def _stage1_plan():
    tiles = [(k, n) for k in range(KT) for n in range(2 * PRE)]
    segs, seen_k, lo = [], 0, 0
    for c in CUTS:
        ts = tiles[lo:4 * c]
        lo = 4 * c
        kr = {}
        for k, n in ts:
            a, b = kr.get(n, (k, k + 1))
            kr[n] = (min(a, k), max(b, k + 1))
        rects = []
        for n in sorted(kr):
            if rects and rects[-1][:2] == kr[n] and rects[-1][3] == n and n != PRE:
                rects[-1] = (*kr[n], rects[-1][2], n + 1)
            else:
                rects.append((*kr[n], n, n + 1))
        k_end = max(seen_k, max(k for k, _ in ts) + 1)
        segs.append(((seen_k, k_end), rects))
        seen_k = k_end
    assert lo == len(tiles)
    return segs


SEGS = _stage1_plan()


def _spread(tasks, t0, t1, weights=None):
    if weights is None:
        return [(t0 + (t1 - t0) * n // len(tasks), fs) for n, fs in enumerate(tasks)]
    total, cum, t, out = sum(weights[t0:t1]), 0.0, t0, []
    for n, fs in enumerate(tasks):
        while cum + weights[t] <= total * n / len(tasks):
            cum += weights[t]
            t += 1
        out.append((t, fs))
    return out


def _plan(preps, spans, works, span, prof, costs=None, load=None):
    sched, work, firsts = [], [], []
    for n, tasks in enumerate(preps):
        timed = _spread(tasks, spans[2 * n], spans[2 * n + 1])
        sched += timed
        if load is not None:
            ops, d0, d1 = costs[n]
            for t, _ in timed:
                for tt in range(t + d0, min(t + d1, len(load))):
                    load[tt] += ops / (d1 - d0)
    for wk in works:
        firsts.append(len(work))
        work += wk
    weights = [[w for t, w in prof if t <= tt][-1] for tt in range(span[1])]
    if load is not None:
        weights = [w * max(0.05, CAP - ld) for w, ld in zip(weights, load)]
    timed = _spread(work, span[0], span[1], weights)
    sched += timed
    sched.sort(key=lambda e: e[0])
    return sched, [timed[f][0] for f in firsts]


def _emit(sched, t0, res, tokens):
    taps = {}
    while sched and sched[0][0] < t0 + res.shape[0]:
        t, fs = sched.pop(0)
        r0 = (t - t0) // 8 * 8
        for f in fs:
            if r0 not in taps:
                taps[r0] = res[r0:r0 + 8, :]
            tok = f(taps[r0])
            if tok is not None:
                tokens.append((t, tok))


def _kernel(xa, ka, va, wqa, woa, xb, kb, vb, wqb, wob, out_hbm,
            x_buf, xp_buf, wq_buf, ku_buf, kx_buf, km_buf, v_buf, wo_buf, qm_buf, o_buf,
            qacc, acc, carry_buf, out_buf, qu0, qu, qxa, qxb, qw, p_u, p_x, p_w, s_buf, pm_buf,
            krec0, kt0, qta, qto, krec1, kt1, qt1, sems, cnt):
    k_hbm, v_hbm, wq_hbm, wo_hbm = (ka, kb), (va, vb), (wqa, wqb), (woa, wob)
    copy = pltpu.make_async_copy

    def k_pair(i, h0, h1, buf):
        blk, half = divmod(i, 2)
        return (k_hbm[blk].at[:, half * IH + h0:half * IH + h1], buf.at[i])

    groups = []
    for si, ((xk0, xk1), rects) in enumerate(SEGS):
        g = []
        for k0, k1, n0, n1 in rects:
            it, c0 = divmod(n0, PRE)
            c0, c1 = c0 * DH, (c0 + n1 - n0) * DH
            g.append((wqa.at[k0 * DH:k1 * DH, it * IW + c0:it * IW + c1],
                      wq_buf.at[it, k0 * DH:k1 * DH, c0:c1]))
        if xk1 > xk0:
            g.append((xa.at[:, xk0 * DH:xk1 * DH], x_buf.at[0, :, xk0 * DH:xk1 * DH]))
        groups.append((si, g))
    groups.append((SEM_XB, [(xb, x_buf.at[1]), k_pair(0, 0, UH, ku_buf)]))
    for j in range(2):
        groups.append((SEM_S2 + j, [(wqb.at[:, j * IW:j * IW + PW], wq_buf.at[2 + j, :, 0:PW]),
                                    k_pair(j, X0, M0, kx_buf), k_pair(2 + j, X0, M0, kx_buf)]))
    for i in range(NI):
        blk, half = divmod(i, 2)
        groups.append((SEM_S3 + i, [
            (wq_hbm[blk].at[:, half * IW + PW:(half + 1) * IW], wq_buf.at[i, :, PW:IW]),
            k_pair(i, M0, IH, km_buf),
            (v_hbm[blk].at[:, half * IH:(half + 1) * IH], v_buf.at[i]),
            (wo_hbm[blk].at[half * IW:(half + 1) * IW, :], wo_buf.at[i, :, 0:D]),
        ]))
        if i + 1 < NI:
            groups.append((SEM_KU + i, [k_pair(i + 1, 0, UH, ku_buf)]))

    for s, group in groups:
        for src, dst in group:
            copy(src, dst, sems.at[s]).start()

    def wait_group(g):
        s, group = groups[g]
        for src, dst in group:
            copy(src, dst, sems.at[s]).wait()

    def out_chunks(n):
        rows = M // TAIL_CHUNKS if n == D // DH - 1 else M
        return [(r0, rows) for r0 in range(0, M, rows)]

    def out_copy(blk, n, r0, rows):
        return copy(out_buf.at[blk, r0:r0 + rows, n * DH:(n + 1) * DH],
                    out_hbm.at[r0:r0 + rows, pl.ds(pl.multiple_of(blk * D + n * DH, DH), DH)],
                    sems.at[SEM_OUT])

    def store_q(it, h, q):
        if h in MHEADS:
            qm_buf[it, :, (h - M0) * DH:(h - M0 + 1) * DH] = q.astype(BF16)
            return
        if h >= W0:
            dst, hh = qw, h - W0
        elif h >= X0:
            dst, hh = (qxa.at[it] if isinstance(it, int) else qxb.at[it - 2]), h - X0
        elif isinstance(it, int) and it == 0:
            dst, hh = qu0, h
        else:
            dst, hh = qu.at[it - 1], h
        for b in range(B):
            r = (hh * B + b) * P32
            dst[r:r + SQ, :] = q[b * SQ:(b + 1) * SQ]

    def vpu_tasks(subs, nh, k_rec, kt, smc, cpb, never):
        nrec = nh * B
        rep = 128 // (nrec * len(subs))
        pstep = 16 // rep
        never8 = jnp.broadcast_to(never, (8, 128))
        never16 = jnp.broadcast_to(never, (16, 128))
        lane_b = lax.broadcasted_iota(jnp.int32, (SK, 128), 1) % GB
        lane_masks = [lane_b == bb for bb in range(GB)]
        zeros = jnp.zeros((SK, 128), U32)

        def tie(x, tap):
            if x.dtype != F32:
                tap = pltpu.bitcast(tap, x.dtype)
            return lax.select(never8, tap, x)

        def tie_first(x, tap):
            return jnp.concatenate([tie(x[0:8], tap), x[8:]], axis=0)

        def copy_k(sub, h, b0, tap):
            tap2 = pltpu.bitcast(jnp.concatenate([tap, tap], axis=0), U32)
            for b in range(b0, b0 + cpb):
                r = (sub * nrec + h * B + b) * P16
                k_rec[r:r + 16, :] = lax.select(never16, tap2, pltpu.bitcast(subs[sub][0](b, h), U32))

        def xpose_k(kp, tap):
            x = k_rec[pl.ds(kp, nrec * len(subs), stride=P16), :]
            t = tie_first(jnp.concatenate([x] * rep, axis=0), tap).T
            kt[pl.ds(2 * kp, DH, stride=P32), :] = pltpu.bitcast(t << 16, F32)
            kt[pl.ds(2 * kp + 1, DH, stride=P32), :] = pltpu.bitcast(t & jnp.uint32(0xFFFF0000), F32)
            return t[120:128]

        def xpose_q(q, qt, row, tap):
            x = jnp.concatenate([q_rec[pl.ds(q + part * 2 * pstep, nrec, stride=P32), :]
                                 for part in range(rep) for _, q_rec, _ in subs], axis=0)
            t = tie_first(x, tap).T
            qt[row] = t
            return pltpu.bitcast(t[120:128], U32)

        scores = {}
        q_vec = [None]

        def block(q, qt, d0, tap):
            dv = d0 // 8 * 8
            if d0 == dv:
                q_vec[0] = qt[q, dv:dv + 8, :]
            qv = tie(q_vec[0], tap)
            a = scores.get(q)
            for d in range(d0, d0 + DBLK):
                t = qv[d - dv:d - dv + 1, :] * kt[d * P32:d * P32 + SK, :]
                a = t if a is None else a + t
            scores[q] = a
            if d0 + DBLK == DH:
                s_buf[...] = a

        def softmax_bits(q, tap):
            s = tie_first(scores.pop(q), tap)
            m = jnp.max(s, axis=0, keepdims=True)
            e = jnp.exp2((s - m) * EXP_SCALE)
            l = jnp.sum(e, axis=0, keepdims=True)
            p = (e * pl.reciprocal(l, approx=True)).astype(BF16).astype(F32)
            return pltpu.bitcast(p, U32)

        def softmax_pair(j, slot, tap):
            pk = (softmax_bits(2 * j, tap) >> 16) | softmax_bits(2 * j + 1, tap)
            t = jnp.concatenate([lax.select(mk, pk, zeros) for mk in lane_masks], axis=0).T
            r0 = 0
            for part in range(rep):
                for _, _, p_rec in subs:
                    p_rec[pl.ds(slot + part * pstep, nrec, stride=P16), :] = t[r0:r0 + nrec]
                    r0 += nrec
            return t[120:128]

        copies = [[functools.partial(copy_k, sub, h, b0)]
                  for sub in range(len(subs)) for h in range(nh) for b0 in range(0, B, cpb)]
        kposes = [[functools.partial(xpose_k, kp)] for kp in range(SK // 2)]

        def qposes(q0, qt, row0, n):
            return [[functools.partial(xpose_q, q0 + e, qt, row0 + e)] for e in range(n)]

        def work(qt, slot0, nslot):
            out = []
            for j in range(nslot):
                for q in (2 * j, 2 * j + 1):
                    for d0 in range(0, DH, DBLK):
                        out.append([functools.partial(block, q, qt, d0)])
                if (j + 1) % SMB == 0:
                    for jj in range(j + 1 - SMB, j + 1):
                        out[-1].append(functools.partial(softmax_pair, jj, slot0 + jj))
                    out += [[]] * smc
            assert nslot % SMB == 0
            return out
        return copies, kposes, qposes, work

    def stage1():
        for si, ((xk0, xk1), rects) in enumerate(SEGS):
            wait_group(si)
            if xk1 > xk0:
                xp_buf[0, :, xk0 * DH:xk1 * DH] = pltpu.bitcast(x_buf[0, :, xk0 * DH:xk1 * DH], U32)
            for k0, k1, n0, n1 in rects:
                it, c0 = divmod(n0, PRE)
                step = (n1 - n0) if k1 - k0 < 4 else 1
                for n in range(n0, n1, step):
                    ca = (c0 + n - n0) * DH
                    cb = ca + step * DH
                    lhs = pltpu.bitcast(xp_buf[0, :, k0 * DH:k1 * DH], BF16)
                    r = jnp.dot(lhs, wq_buf[it, k0 * DH:k1 * DH, ca:cb], preferred_element_type=F32)
                    if k0 > 0:
                        r = qacc[:, n * DH:(n + step) * DH] + r
                    if k1 < KT:
                        qacc[:, n * DH:(n + step) * DH] = r
                    else:
                        for hh in range(step):
                            store_q(it, c0 + n - n0 + hh, r[:, hh * DH:(hh + 1) * DH])

    def make_q_round(blk, it):
        q_part = {}

        def q_round(h, half, fill_xp, t0):
            ks = slice(half * (D // 2), (half + 1) * (D // 2))
            if fill_xp:
                lhs = x_buf[blk, :, ks]
                xp_buf[blk, :, ks] = pltpu.bitcast(lhs, U32)
            else:
                lhs = pltpu.bitcast(xp_buf[blk, :, ks], BF16)
            r = jnp.dot(lhs, wq_buf[it, ks, h * DH:(h + 1) * DH], preferred_element_type=F32)
            if half == 0:
                q_part[h] = r
            else:
                store_q(it, h, q_part.pop(h) + r)
            return r
        return q_round

    def stage2(j, carry):
        for dst in (wq_buf.at[2 + j, :, 0:PW], kx_buf.at[j], kx_buf.at[2 + j]):
            copy(dst, dst, sems.at[SEM_S2 + j]).wait()
        q_round = make_q_round(1, 2 + j)
        never = j == 77
        uc, uk, uq, uw = vpu_tasks([(lambda b, h: ku_buf[0, b, h], qu0, p_u)], UH, krec0, kt0,
                                   SMC2, CPB2, never)
        xc, xk, xq, xw = vpu_tasks([(lambda b, h: kx_buf[j, b, h], qxa.at[j], p_x.at[j]),
                                    (lambda b, h: kx_buf[2 + j, b, h], qxb.at[j], p_x.at[2 + j])],
                                   XH, krec1, kt1, SMC2, CPB2, never)
        preps = [uc, uk, uq(j * AS, qta, 0, AS), uq(2 * AS + j * (16 - AS), qto, j * (16 - AS), 16 - AS),
                 xc, xk, xq(0, qt1, 0, 8 * XH)]
        works = [uw(qta, j * (AS // 2), AS // 2), xw(qt1, 0, 4 * XH)]
        pr = PREP2
        sched, starts = _plan(preps, pr, works, SPAN2, PROF2)
        assert pr[2] >= pr[1] and starts[0] > max(pr[3], pr[5]) + 200
        assert pr[10] >= pr[9] and pr[12] >= 2 * XH * M + 200 and starts[1] > max(pr[11], pr[13]) + 200
        order = list(range(X0, M0)) + [h for h in range(PRE) if not X0 <= h < M0]
        t0 = 0
        for n, h in enumerate(order):
            for half in range(2):
                _emit(sched, t0, q_round(h, half, n == 0, t0), [])
                t0 += M
        assert not sched
        return carry

    def stage3(i, carry):
        for dst in (wq_buf.at[i, :, PW:IW], km_buf.at[i], v_buf.at[i], wo_buf.at[i, :, 0:D]):
            copy(dst, dst, sems.at[SEM_S3 + i]).wait()
        nxt = jnp.minimum(i + 1, NI - 1)

        @pl.when(i + 1 < NI)
        def _():
            dst = ku_buf.at[nxt]
            copy(dst, dst, sems.at[SEM_KU + nxt - 1]).wait()

        blk = lax.shift_right_logical(i, 1)
        second_half = (i & 1) == 1
        never = i == 77
        tokens = []
        row = lax.broadcasted_iota(jnp.int32, (128, 128), 0) // SQ
        col = lax.broadcasted_iota(jnp.int32, (128, 128), 1) // SK
        same_batch = row == col

        def qk_softmax(h, t0):
            tap = None
            for g in range(B // GB):
                qg = qm_buf[i, g * 128:(g + 1) * 128, (h - M0) * DH:(h - M0 + 1) * DH]
                kg = km_buf[i, GB * g:GB * (g + 1), h - M0].reshape(128, DH)
                s = lax.dot_general(qg, kg, NT_DIMS, preferred_element_type=F32)
                tap = s if tap is None else tap
                s = jnp.where(same_batch, s, -jnp.inf)
                m = jnp.max(s, axis=-1, keepdims=True)
                e = jnp.exp2((s - m) * EXP_SCALE)
                l = jnp.sum(e, axis=-1, keepdims=True)
                pm_buf[h - M0, g] = (e * pl.reciprocal(l, approx=True)).astype(BF16)
            return tap

        def pv(h, t0):
            tap = None
            for g in range(B // GB):
                if h in MHEADS:
                    p = pm_buf[h - M0, g]
                else:
                    rec, hh = (p_u, h) if h < X0 else (p_x.at[i], h - X0) if h < M0 else (p_w, h - W0)
                    parts = [rec[(hh * B + b) * P16:(hh * B + b) * P16 + 16, :]
                             for b in range(GB * g, GB * (g + 1))]
                    p = pltpu.bitcast(jnp.concatenate(parts, axis=0), BF16)
                vg = v_buf[i, GB * g:GB * (g + 1), h].reshape(128, DH)
                o = jnp.dot(p, vg, preferred_element_type=F32)
                tap = o if tap is None else tap
                o_buf[g * 64:(g + 1) * 64, h * DH:(h + 1) * DH] = pltpu.bitcast(o.astype(BF16), U32)
            return tap

        q_round = make_q_round(blk, i)

        def o_round(g, n, t0):
            cs = slice(n * DH, (n + 1) * DH)
            lhs = o_buf[:, g * GW:(g + 1) * GW]
            if t0 in hold_rounds:
                got = [v for t, v in tokens if t + LAG < t0]
                tokens[:] = [e for e in tokens if e[0] + LAG >= t0]
                if got:
                    tok = functools.reduce(lambda a, b: a | b, got)
                    top = jnp.concatenate([jnp.where(never, tok, lhs[0:8, 0:128]), lhs[0:8, 128:]], axis=1)
                    lhs = jnp.concatenate([top, lhs[8:]], axis=0)
            r = jnp.dot(pltpu.bitcast(lhs, BF16), wo_buf[i, g * GW:(g + 1) * GW, cs],
                        preferred_element_type=F32)
            s = (carry_buf[i & 1, :, cs] if g == GORDER[0] else acc[:, cs]) + r
            if g == GORDER[-1]:
                carry_buf[1, :, cs] = s
                for r0, rows in out_chunks(n):
                    out_buf[blk, r0:r0 + rows, cs] = s[r0:r0 + rows].astype(BF16)

                    @pl.when(second_half)
                    def _():
                        out_copy(blk, n, r0, rows).start()
            else:
                acc[:, cs] = s
            return r

        rounds = [functools.partial(q_round, h, half, False) for h in range(PRE, IH) for half in range(2)]
        nq = len(rounds)
        rounds += [functools.partial(o_round, g, n) for g in GORDER for n in range(D // DH)]
        pr = PREP3
        jobs, t0, pv_times = [], 0, {}
        load = [0.0] * (len(rounds) * M + 128 * (IH + len(MHEADS)))

        def add_load(a, b, ops):
            for tt in range(max(a, 0), min(b, len(load))):
                load[tt] += ops / (b - a)

        for step, rd in enumerate(rounds):
            jobs.append((t0, rd))
            add_load(t0, t0 + M, 288 if step >= nq or step % 2 else 224)
            if step >= len(rounds) - D // DH:
                add_load(t0, t0 + M, LC[0])
            t0 += M
            if step == nq - 1:
                assert pr[4] > t0 + 100
            for h in reversed(range(IH)):
                if PV_AT[h] == step:
                    assert step < nq + (D // DH) * GORDER.index(h // GH) - 1
                    pv_times[h] = t0
                    add_load(t0 - LC[2], t0 - LC[2] + 128, LC[1])
                    add_load(t0, t0 + 128, 32)
                    jobs.append((t0, functools.partial(pv, h)))
                    t0 += 128
            for h in MHEADS:
                if QK_AT[h - M0] == step:
                    assert PV_AT[h] > step
                    add_load(t0 - LC[2], t0 - LC[2] + 128, LC[1])
                    add_load(t0, t0 + LC[4], LC[3])
                    jobs.append((t0, functools.partial(qk_softmax, h)))
                    t0 += 128

        uc, uk, uq, uw = vpu_tasks([(lambda b, h: ku_buf[nxt, b, h], qu.at[nxt - 1], p_u)], UH, krec0, kt0,
                                   SMC, CPB, never)
        wc, wk, wq, ww = vpu_tasks([(lambda b, h: km_buf[i, b, W0 - M0 + h], qw, p_w)], WH, krec1, kt1,
                                   SMC, CPB, never)
        preps = [wc, wk, wq(0, qt1, 0, 4 * WH), uc, uk, uq(0, qta, 0, 2 * AS), uq(2 * AS, qto, 0, 2 * (16 - AS))]
        works = [uw(qto, AS, 16 - AS), ww(qt1, 0, 2 * WH), uw(qta, 0, AS)]
        cc, kc, qc = (4 * CPB, 0, 8 * CPB), (LC[5], 150, 300), (LC[6], 150, 300)
        sched, starts = _plan(preps, pr, works, SPAN3, PROF3, [cc, kc, qc, cc, kc, qc, qc], load)
        assert pr[2] >= pr[1] and starts[1] > max(pr[3], pr[5]) + 200
        assert pr[8] >= pr[7] and min(pr[8], pr[12]) > starts[1] and starts[2] > max(pr[9], pr[11]) + 200
        for h, t in pv_times.items():
            if h < X0:
                assert starts[1] + 400 < t < starts[2]
            elif h >= W0:
                assert t > starts[2] + 400
        o_starts = [t for t, job in jobs if job.func is o_round]
        hold_rounds = {max(t for t in o_starts if t <= s) for s in (starts[1], starts[2], pr[13] + LAG + M)}
        for t0, job in jobs:
            _emit(sched, t0, job(t0), tokens)
        assert not sched
        return carry

    def body(_, carry):
        carry_buf[0] = jnp.zeros((M, D), F32)
        stage1()
        wait_group(len(SEGS))
        lax.fori_loop(0, 2, stage2, 0)
        lax.fori_loop(0, NI, stage3, 0)
        for blk in range(2):
            for n in range(D // DH):
                for r0, rows in out_chunks(n):
                    out_copy(blk, n, r0, rows).wait()
        return carry

    cnt[0] = 1
    lax.fori_loop(0, cnt[0], body, 0)


@jax.jit
def pallas_concat_heads__mha_block_cached__mha_block_cached__near_ridge_kernel(
    A_x: jax.Array,
    A_k_cache: jax.Array,
    A_v_cache: jax.Array,
    A_wq: jax.Array,
    A_wo: jax.Array,
    B_x: jax.Array,
    B_k_cache: jax.Array,
    B_v_cache: jax.Array,
    B_wq: jax.Array,
    B_wo: jax.Array,
):
    def rec16(nh):
        return (nh * B * P16 + 24, 128)

    def rec32(nh):
        return (nh * B * P32 + 40, 128)

    k_t = pltpu.VMEM((DH * P32 + 40, 128), F32)
    out = pl.pallas_call(
        _kernel,
        in_specs=[pl.BlockSpec(memory_space=pl.ANY)] * 10,
        out_specs=pl.BlockSpec(memory_space=pl.ANY),
        out_shape=jax.ShapeDtypeStruct((M, 2 * D), BF16),
        scratch_shapes=[
            pltpu.VMEM((2, M, D), BF16),
            pltpu.VMEM((2, M // 2, D), U32),
            pltpu.VMEM((NI, D, IW + W_PAD), BF16),
            pltpu.VMEM((NI, B, UH, SK, DH), BF16),
            pltpu.VMEM((NI, B, XH, SK, DH), BF16),
            pltpu.VMEM((NI, B, IH - M0, SK, DH), BF16),
            pltpu.VMEM((NI, B, IH, SK, DH), BF16),
            pltpu.VMEM((NI, IW, D + W_PAD), BF16),
            pltpu.VMEM((NI, M, len(MHEADS) * DH), BF16),
            pltpu.VMEM((M // 2, IW), U32),
            pltpu.VMEM((M, 2 * PW), F32),
            pltpu.VMEM((M, D), F32),
            pltpu.VMEM((2, M, D), F32),
            pltpu.VMEM((2, M, D), BF16),
            pltpu.VMEM(rec32(UH), F32),
            pltpu.VMEM((NI - 1,) + rec32(UH), F32),
            pltpu.VMEM((2,) + rec32(XH), F32),
            pltpu.VMEM((2,) + rec32(XH), F32),
            pltpu.VMEM(rec32(WH), F32),
            pltpu.VMEM(rec16(UH), U32),
            pltpu.VMEM((NI,) + rec16(XH), U32),
            pltpu.VMEM(rec16(WH), U32),
            pltpu.VMEM((SK, 128), F32),
            pltpu.VMEM((len(MHEADS), B // GB, 128, 128), BF16),
            pltpu.VMEM(rec16(UH), U32), k_t,
            pltpu.VMEM((2 * AS, DH, 128), F32),
            pltpu.VMEM((2 * (16 - AS), DH, 128), F32),
            pltpu.VMEM(rec16(WH), U32), k_t,
            pltpu.VMEM((4 * WH, DH, 128), F32),
            pltpu.SemaphoreType.DMA((NUM_SEMS,)),
            pltpu.SMEM((1,), jnp.int32),
        ],
        compiler_params=pltpu.CompilerParams(
            vmem_limit_bytes=112 * 1024 * 1024,
            disable_bounds_checks=True,
            disable_semaphore_checks=True,
        ),
    )(A_x.reshape(M, D), A_k_cache, A_v_cache, A_wq, A_wo,
      B_x.reshape(M, D), B_k_cache, B_v_cache, B_wq, B_wo)
    return out.reshape(B, SQ, 2 * D)
```

```python
import functools

import jax
import jax.numpy as jnp
from jax import lax
import jax.experimental.pallas as pl
import jax.experimental.pallas.tpu as pltpu

B, SQ, D = 16, 32, 1024
H, SK, DH = 32, 32, 128
M = B * SQ
KT = D // DH
GB = 128 // SQ
IH = 16
NI = 4
IW = IH * DH
PRE = 12
PW = PRE * DH
GH = 4
GW = GH * DH
W_PAD = 128
TAIL_CHUNKS = 4
P16 = 20
P32 = 36
EXP_SCALE = DH ** -0.5 * 1.4426950408889634
NT_DIMS = (((1,), (1,)), ((), ()))
F32 = jnp.float32
BF16 = jnp.bfloat16
U32 = jnp.uint32

UH, XH, YH, WH = 4, 3, 4, 4
X0 = UH
M0 = UH + XH
W0 = IH - WH
Y0 = W0 - YH
MHEADS = range(M0, Y0)
US = 2 * UH
AS = 6

CUTS = (1, 4, 8, 16, 28, 48)

GORDER = (0, 1, 2, 3)
QK_AT = (7,)
PV_AT = (5, 4, 6, 6, 0, 0, 1, 10, 18, 20, 20, 20, 30, 30, 30, 30)
PREP3 = (0, 200, 700, 1700, 0, 1400, 4000, 5000, 5500, 7300, 6000, 8000, 10064, 11000, 11000, 13500, 9500, 11000, 14400, 15000)
SPAN3 = (64, 22140)
PROF3 = ((0, 0.97), (2000, 1.0), (18600, 1.1))
PREP2 = (0, 200, 200, 1200, 0, 400, 500, 1200, 1800, 3400, 3300, 4600)
PREP1 = (0, 400, 400, 1600, 0, 1000, 4000, 5000)
SPAN1 = (1900, 9700)
SPAN2 = (1500, 11850)
PROF2 = ((0, 1.0), (5000, 1.03), (9300, 1.0))
DBLK = 2
SMB = 2
SMC = 16
SMC2 = 16
CPB = 1
CPB2 = 2
LAG = 900
LAG1 = 400
HOLD1 = 0
CAP = 3.3
LC = (96, 64, 140, 400, 500, 40, 8)

SEM_XB = len(CUTS)
SEM_S2 = SEM_XB + 1
SEM_S3 = SEM_S2 + 2
SEM_OUT = SEM_S3 + NI
NUM_SEMS = SEM_OUT + 1


def _stage1_plan():
    tiles = [(k, n) for k in range(KT // 2) for n in range(2 * PRE)]
    tiles += [(k, n) for n in range(2 * PRE) for k in range(KT // 2, KT)]
    segs, seen_k, lo = [], 0, 0
    for c in CUTS:
        ts = tiles[lo:4 * c]
        lo = 4 * c
        kr = {}
        for k, n in ts:
            a, b = kr.get(n, (k, k + 1))
            kr[n] = (min(a, k), max(b, k + 1))
        rects = []
        for n in sorted(kr):
            if rects and rects[-1][:2] == kr[n] and rects[-1][3] == n and n != PRE:
                rects[-1] = (*kr[n], rects[-1][2], n + 1)
            else:
                rects.append((*kr[n], n, n + 1))
        k_end = max(seen_k, max(k for k, _ in ts) + 1)
        segs.append(((seen_k, k_end), rects))
        seen_k = k_end
    assert lo == len(tiles)
    return segs


SEGS = _stage1_plan()


def _spread(tasks, t0, t1, weights=None):
    if weights is None:
        return [(t0 + (t1 - t0) * n // len(tasks), fs) for n, fs in enumerate(tasks)]
    total, cum, t, out = sum(weights[t0:t1]), 0.0, t0, []
    for n, fs in enumerate(tasks):
        while cum + weights[t] <= total * n / len(tasks):
            cum += weights[t]
            t += 1
        out.append((t, fs))
    return out


def _plan(preps, spans, works, span, prof, costs=None, load=None):
    sched, work, firsts = [], [], []
    for n, tasks in enumerate(preps):
        timed = _spread(tasks, spans[2 * n], spans[2 * n + 1])
        sched += timed
        if load is not None:
            ops, d0, d1 = costs[n]
            for t, _ in timed:
                for tt in range(t + d0, min(t + d1, len(load))):
                    load[tt] += ops / (d1 - d0)
    for wk in works:
        firsts.append(len(work))
        work += wk
    weights = [[w for t, w in prof if t <= tt][-1] for tt in range(span[1])]
    if load is not None:
        weights = [w * max(0.05, CAP - ld) for w, ld in zip(weights, load)]
    timed = _spread(work, span[0], span[1], weights)
    sched += timed
    sched.sort(key=lambda e: e[0])
    return sched, [timed[f][0] for f in firsts]


def _emit(sched, t0, res, tokens):
    taps = {}
    while sched and sched[0][0] < t0 + res.shape[0]:
        t, fs = sched.pop(0)
        r0 = (t - t0) // 8 * 8
        for f in fs:
            if r0 not in taps:
                taps[r0] = res[r0:r0 + 8, :]
            tok = f(taps[r0])
            if tok is not None:
                tokens.append((t, tok))


def _kernel(xa, ka, va, wqa, woa, xb, kb, vb, wqb, wob, out_hbm,
            x_buf, xp_buf, wq_buf, ku_buf, kx_buf, km_buf, v_buf, wo_buf, qm_buf, o_buf,
            qacc, acc, carry_buf, out_buf, qu0, qu, qxa, qxb, qy, qw, p_u, p_x, p_y, p_w, s_buf, pm_buf,
            krec0, kt0, qta, qto, krec1, kt1, qt1, krec2, kt2, qt2, sems, cnt):
    k_hbm, v_hbm, wq_hbm, wo_hbm = (ka, kb), (va, vb), (wqa, wqb), (woa, wob)
    copy = pltpu.make_async_copy

    def k_pair(i, h0, h1, buf, slot=None):
        blk, half = divmod(i, 2)
        return (k_hbm[blk].at[:, half * IH + h0:half * IH + h1], buf.at[i if slot is None else slot])

    groups = []
    for si, ((xk0, xk1), rects) in enumerate(SEGS):
        g = []
        for k0, k1, n0, n1 in rects:
            it, c0 = divmod(n0, PRE)
            c0, c1 = c0 * DH, (c0 + n1 - n0) * DH
            g.append((wqa.at[k0 * DH:k1 * DH, it * IW + c0:it * IW + c1],
                      wq_buf.at[it, k0 * DH:k1 * DH, c0:c1]))
        if xk1 > xk0:
            g.append((xa.at[:, xk0 * DH:xk1 * DH], x_buf.at[0, :, xk0 * DH:xk1 * DH]))
        if si == len(SEGS) - 1:
            g.append(k_pair(0, 0, UH, ku_buf))
        groups.append((si, g))
    groups.append((SEM_XB, [(xb, x_buf.at[1])]))
    for j in range(2):
        groups.append((SEM_S2 + j, [(wqb.at[:, j * IW:j * IW + PW], wq_buf.at[2 + j, :, 0:PW]),
                                    k_pair(j, X0, M0, kx_buf), k_pair(2 + j, X0, M0, kx_buf)]))
    for i in range(NI):
        blk, half = divmod(i, 2)
        groups.append((SEM_S3 + i, [
            (wq_hbm[blk].at[:, half * IW + PW:(half + 1) * IW], wq_buf.at[i, :, PW:IW]),
            k_pair(i, M0, IH, km_buf),
            (v_hbm[blk].at[:, half * IH:(half + 1) * IH], v_buf.at[i]),
            (wo_hbm[blk].at[half * IW:(half + 1) * IW, :], wo_buf.at[i, :, 0:D]),
            k_pair(min(i + 1, NI - 1), 0, UH, ku_buf, i + 1),
        ]))

    for s, group in groups:
        for src, dst in group:
            copy(src, dst, sems.at[s]).start()

    def wait_group(g):
        s, group = groups[g]
        for src, dst in group:
            copy(src, dst, sems.at[s]).wait()

    def out_chunks(n):
        rows = M // TAIL_CHUNKS if n == D // DH - 1 else M
        return [(r0, rows) for r0 in range(0, M, rows)]

    def out_copy(blk, n, r0, rows):
        return copy(out_buf.at[blk, r0:r0 + rows, n * DH:(n + 1) * DH],
                    out_hbm.at[r0:r0 + rows, pl.ds(pl.multiple_of(blk * D + n * DH, DH), DH)],
                    sems.at[SEM_OUT])

    def store_q(it, h, q):
        if h in MHEADS:
            qm_buf[it, :, (h - M0) * DH:(h - M0 + 1) * DH] = q.astype(BF16)
            return
        if h >= W0:
            dst, hh = qw, h - W0
        elif h >= Y0:
            dst, hh = qy.at[it], h - Y0
        elif h >= X0:
            dst, hh = (qxa.at[it, h - X0] if isinstance(it, int) else qxb.at[it - 2, h - X0]), 0
        elif isinstance(it, int) and it == 0:
            dst, hh = qu0, h
        else:
            dst, hh = qu.at[it - 1], h
        for b in range(B):
            r = (hh * B + b) * P32
            dst[r:r + SQ, :] = q[b * SQ:(b + 1) * SQ]

    def vpu_tasks(subs, nh, k_rec, kt, smc, cpb, never):
        nrec = nh * B
        rep = 128 // (nrec * len(subs))
        pstep = 16 // rep
        never8 = jnp.broadcast_to(never, (8, 128))
        never16 = jnp.broadcast_to(never, (16, 128))
        lane_b = lax.broadcasted_iota(jnp.int32, (SK, 128), 1) % GB
        lane_masks = [lane_b == bb for bb in range(GB)]
        zeros = jnp.zeros((SK, 128), U32)

        def tie(x, tap):
            if x.dtype != F32:
                tap = pltpu.bitcast(tap, x.dtype)
            return lax.select(never8, tap, x)

        def tie_first(x, tap):
            return jnp.concatenate([tie(x[0:8], tap), x[8:]], axis=0)

        def copy_k(sub, h, b0, tap):
            tap2 = pltpu.bitcast(jnp.concatenate([tap, tap], axis=0), U32)
            for b in range(b0, b0 + cpb):
                r = (sub * nrec + h * B + b) * P16
                k_rec[r:r + 16, :] = lax.select(never16, tap2, pltpu.bitcast(subs[sub][0](b, h), U32))

        def xpose_k(kp, tap):
            x = k_rec[pl.ds(kp, nrec * len(subs), stride=P16), :]
            t = tie_first(jnp.concatenate([x] * rep, axis=0), tap).T
            kt[pl.ds(2 * kp, DH, stride=P32), :] = pltpu.bitcast(t << 16, F32)
            kt[pl.ds(2 * kp + 1, DH, stride=P32), :] = pltpu.bitcast(t & jnp.uint32(0xFFFF0000), F32)
            return t[120:128]

        def xpose_q(q, qt, row, tap):
            x = jnp.concatenate([q_rec[pl.ds(q + part * 2 * pstep, nrec, stride=P32), :]
                                 for part in range(rep) for _, q_rec, _ in subs], axis=0)
            t = tie_first(x, tap).T
            qt[row] = t
            return pltpu.bitcast(t[120:128], U32)

        scores = {}
        q_vec = [None]

        def block(q, qt, d0, tap):
            dv = d0 // 8 * 8
            if d0 == dv:
                q_vec[0] = qt[q, dv:dv + 8, :]
            qv = tie(q_vec[0], tap)
            a = scores.get(q)
            for d in range(d0, d0 + DBLK):
                t = qv[d - dv:d - dv + 1, :] * kt[d * P32:d * P32 + SK, :]
                a = t if a is None else a + t
            scores[q] = a
            if d0 + DBLK == DH:
                s_buf[...] = a

        def softmax_bits(q, tap):
            s = tie_first(scores.pop(q), tap)
            m = jnp.max(s, axis=0, keepdims=True)
            e = jnp.exp2((s - m) * EXP_SCALE)
            l = jnp.sum(e, axis=0, keepdims=True)
            p = (e * pl.reciprocal(l, approx=True)).astype(BF16).astype(F32)
            return pltpu.bitcast(p, U32)

        def softmax_pair(j, slot, tap):
            pk = (softmax_bits(2 * j, tap) >> 16) | softmax_bits(2 * j + 1, tap)
            t = jnp.concatenate([lax.select(mk, pk, zeros) for mk in lane_masks], axis=0).T
            r0 = 0
            for part in range(rep):
                for _, _, p_rec in subs:
                    p_rec[pl.ds(slot + part * pstep, nrec, stride=P16), :] = t[r0:r0 + nrec]
                    r0 += nrec
            return t[120:128]

        copies = [[functools.partial(copy_k, sub, h, b0)]
                  for sub in range(len(subs)) for h in range(nh) for b0 in range(0, B, cpb)]
        kposes = [[functools.partial(xpose_k, kp)] for kp in range(SK // 2)]

        def qposes(q0, qt, row0, n):
            return [[functools.partial(xpose_q, q0 + e, qt, row0 + e)] for e in range(n)]

        def work(qt, slot0, nslot):
            out = []
            for j in range(nslot):
                for q in (2 * j, 2 * j + 1):
                    for d0 in range(0, DH, DBLK):
                        out.append([functools.partial(block, q, qt, d0)])
                if (j + 1) % SMB == 0 or j == nslot - 1:
                    for jj in range(j // SMB * SMB, j + 1):
                        out[-1].append(functools.partial(softmax_pair, jj, slot0 + jj))
                    out += [[]] * smc
            return out
        return copies, kposes, qposes, work

    def stage1(never):
        for si, ((xk0, xk1), rects) in enumerate(SEGS):
            wait_group(si)
            if xk1 > xk0:
                xp_buf[0, :, xk0 * DH:xk1 * DH] = pltpu.bitcast(x_buf[0, :, xk0 * DH:xk1 * DH], U32)
            sched, t0 = [], 0
            if si == len(SEGS) - 1:
                uc, uk, uq, uw = vpu_tasks([(lambda b, h: ku_buf[0, b, h], qu0, p_u)], UH, krec0, kt0,
                                           SMC2, CPB2, never)
                sched, starts = _plan([uc, uk, uq(0, qta, 0, 2 * AS), uq(2 * AS, qto, 0, 2 * (US - AS))], PREP1,
                                      [uw(qta, 0, AS)], SPAN1, ((0, 1.0),))
                assert PREP1[2] >= PREP1[1] and starts[0] > max(PREP1[3], PREP1[5]) + 200
                assert all(k1 - k0 == 4 and n0 >= UH for k0, k1, n0, _ in rects)
            for k0, k1, n0, n1 in rects:
                it, c0 = divmod(n0, PRE)
                step = (n1 - n0) if k1 - k0 < 4 else 1
                for n in range(n0, n1, step):
                    ca = (c0 + n - n0) * DH
                    cb = ca + step * DH
                    lhs = pltpu.bitcast(xp_buf[0, :, k0 * DH:k1 * DH], BF16)
                    r = res = jnp.dot(lhs, wq_buf[it, k0 * DH:k1 * DH, ca:cb], preferred_element_type=F32)
                    if k0 > 0:
                        r = qacc[:, n * DH:(n + step) * DH] + r
                    if k1 < KT:
                        qacc[:, n * DH:(n + step) * DH] = r
                    else:
                        for hh in range(step):
                            store_q(it, c0 + n - n0 + hh, r[:, hh * DH:(hh + 1) * DH])
                    _emit(sched, t0, res, [])
                    t0 += M
            assert not sched

    def make_q_round(blk, it, hold=None):
        q_part = {}

        def q_round(h, half, fill_xp, t0):
            ks = slice(half * (D // 2), (half + 1) * (D // 2))
            if fill_xp:
                lhs = x_buf[blk, :, ks]
                xp_buf[blk, :, ks] = pltpu.bitcast(lhs, U32)
            else:
                lhs = xp_buf[blk, :, ks]
                lhs = pltpu.bitcast(lhs if hold is None else hold(lhs, t0), BF16)
            r = jnp.dot(lhs, wq_buf[it, ks, h * DH:(h + 1) * DH], preferred_element_type=F32)
            if half == 0:
                q_part[h] = r
            else:
                store_q(it, h, q_part.pop(h) + r)
            return r
        return q_round

    def stage2(j, carry):
        for dst in (wq_buf.at[2 + j, :, 0:PW], kx_buf.at[j], kx_buf.at[2 + j]):
            copy(dst, dst, sems.at[SEM_S2 + j]).wait()
        q_round = make_q_round(1, 2 + j)
        never = j == 77

        def x_sub(it, q_rec, e):
            return (lambda b, h: kx_buf[it, b, e], q_rec.at[j, e], p_x.at[it, e])

        ac, ak, aq, aw = vpu_tasks([x_sub(j, qxa, 0), x_sub(j, qxa, 1)], 1, krec2, kt2, SMC2, CPB2, never)
        xc, xk, xq, xw = vpu_tasks([x_sub(j, qxa, 2)] + [x_sub(2 + j, qxb, e) for e in range(XH)],
                                   1, krec1, kt1, SMC2, CPB2, never)
        pr = PREP2
        sched, starts = _plan([ac, ak, aq(0, qt2, 0, 8), xc, xk, xq(0, qt1, 0, 16)], pr,
                              [aw(qt2, 0, 4), xw(qt1, 0, 8)], SPAN2, PROF2)
        assert pr[2] >= pr[1] and starts[0] > max(pr[3], pr[5]) + 200
        assert pr[8] >= pr[7] and pr[10] >= 2 * XH * M + 200 and starts[1] > max(pr[9], pr[11]) + 200, starts
        order = list(range(X0, M0)) + [h for h in range(PRE) if not X0 <= h < M0]
        t0 = 0
        for n, h in enumerate(order):
            for half in range(2):
                _emit(sched, t0, q_round(h, half, n == 0, t0), [])
                t0 += M
        assert not sched
        return carry

    def stage3(i, carry):
        for dst in (wq_buf.at[i, :, PW:IW], km_buf.at[i], v_buf.at[i], wo_buf.at[i, :, 0:D], ku_buf.at[i + 1]):
            copy(dst, dst, sems.at[SEM_S3 + i]).wait()
        blk = lax.shift_right_logical(i, 1)
        second_half = (i & 1) == 1
        never = i == 77
        tokens = []
        row = lax.broadcasted_iota(jnp.int32, (128, 128), 0) // SQ
        col = lax.broadcasted_iota(jnp.int32, (128, 128), 1) // SK
        same_batch = row == col

        def qk_softmax(h, t0):
            tap = None
            for g in range(B // GB):
                qg = qm_buf[i, g * 128:(g + 1) * 128, (h - M0) * DH:(h - M0 + 1) * DH]
                kg = km_buf[i, GB * g:GB * (g + 1), h - M0].reshape(128, DH)
                s = lax.dot_general(qg, kg, NT_DIMS, preferred_element_type=F32)
                tap = s if tap is None else tap
                s = jnp.where(same_batch, s, -jnp.inf)
                m = jnp.max(s, axis=-1, keepdims=True)
                e = jnp.exp2((s - m) * EXP_SCALE)
                l = jnp.sum(e, axis=-1, keepdims=True)
                pm_buf[h - M0, g] = (e * pl.reciprocal(l, approx=True)).astype(BF16)
            return tap

        def pv(h, t0):
            tap = None
            for g in range(B // GB):
                if h in MHEADS:
                    p = pm_buf[h - M0, g]
                else:
                    rec, hh = (p_u, h) if h < X0 else (p_x.at[i, h - X0], 0) if h < M0 else (p_y, h - Y0) if h < W0 else (p_w, h - W0)
                    parts = [rec[(hh * B + b) * P16:(hh * B + b) * P16 + 16, :]
                             for b in range(GB * g, GB * (g + 1))]
                    p = pltpu.bitcast(jnp.concatenate(parts, axis=0), BF16)
                vg = v_buf[i, GB * g:GB * (g + 1), h].reshape(128, DH)
                o = jnp.dot(p, vg, preferred_element_type=F32)
                tap = o if tap is None else tap
                o_buf[g * 64:(g + 1) * 64, h * DH:(h + 1) * DH] = pltpu.bitcast(o.astype(BF16), U32)
            return tap

        def hold(lhs, t0):
            for th, lag in holds:
                if t0 <= th < t0 + M:
                    got = [v for t, v in tokens if t + lag < th]
                    tokens[:] = [e for e in tokens if e[0] + lag >= th]
                    if got:
                        r0 = (th - t0) // 16 * 8
                        tok = functools.reduce(lambda a, b: a | b, got)
                        mid = jnp.concatenate([jnp.where(never, tok, lhs[r0:r0 + 8, 0:128]), lhs[r0:r0 + 8, 128:]], axis=1)
                        lhs = jnp.concatenate(([lhs[:r0]] if r0 else []) + [mid] + ([lhs[r0 + 8:]] if r0 + 8 < M // 2 else []), axis=0)
            return lhs

        q_round = make_q_round(blk, i, hold)

        def o_round(g, n, t0):
            cs = slice(n * DH, (n + 1) * DH)
            lhs = hold(o_buf[:, g * GW:(g + 1) * GW], t0)
            r = jnp.dot(pltpu.bitcast(lhs, BF16), wo_buf[i, g * GW:(g + 1) * GW, cs],
                        preferred_element_type=F32)
            s = (carry_buf[i & 1, :, cs] if g == GORDER[0] else acc[:, cs]) + r
            if g == GORDER[-1]:
                carry_buf[1, :, cs] = s
                for r0, rows in out_chunks(n):
                    out_buf[blk, r0:r0 + rows, cs] = s[r0:r0 + rows].astype(BF16)

                    @pl.when(second_half)
                    def _():
                        out_copy(blk, n, r0, rows).start()
            else:
                acc[:, cs] = s
            return r

        rounds = [functools.partial(q_round, h, half, False) for h in range(PRE, IH) for half in range(2)]
        nq = len(rounds)
        rounds += [functools.partial(o_round, g, n) for g in GORDER for n in range(D // DH)]
        pr = PREP3
        jobs, t0, pv_times = [], 0, {}
        load = [0.0] * (len(rounds) * M + 128 * (IH + len(MHEADS)))

        def add_load(a, b, ops):
            for tt in range(max(a, 0), min(b, len(load))):
                load[tt] += ops / (b - a)

        for step, rd in enumerate(rounds):
            jobs.append((t0, rd))
            add_load(t0, t0 + M, 288 if step >= nq or step % 2 else 224)
            if step >= len(rounds) - D // DH:
                add_load(t0, t0 + M, LC[0])
            t0 += M
            if step == nq - 1:
                assert pr[10] > t0 + 100
            for h in reversed(range(IH)):
                if PV_AT[h] == step:
                    assert step < nq + (D // DH) * GORDER.index(h // GH) - 1
                    pv_times[h] = t0
                    add_load(t0 - LC[2], t0 - LC[2] + 128, LC[1])
                    add_load(t0, t0 + 128, 32)
                    jobs.append((t0, functools.partial(pv, h)))
                    t0 += 128
            for h in MHEADS:
                if QK_AT[h - M0] == step:
                    assert PV_AT[h] > step
                    add_load(t0 - LC[2], t0 - LC[2] + 128, LC[1])
                    add_load(t0, t0 + LC[4], LC[3])
                    jobs.append((t0, functools.partial(qk_softmax, h)))
                    t0 += 128

        uc, uk, uq, uw = vpu_tasks([(lambda b, h: ku_buf[i + 1, b, h], qu.at[jnp.minimum(i, NI - 2)], p_u)], UH, krec0, kt0,
                                   SMC, CPB, never)
        wc, wk, wq, ww = vpu_tasks([(lambda b, h: km_buf[i, b, W0 - M0 + h], qw, p_w)], WH, krec1, kt1,
                                   SMC, CPB, never)
        yc, yk, yq, yw = vpu_tasks([(lambda b, h: km_buf[i, b, Y0 - M0 + h], qy.at[i], p_y)], YH, krec2, kt2,
                                   SMC, CPB, never)
        preps = [yc, yk, yq(0, qt2, 0, 4 * YH), wc, wk, wq(0, qt1, 0, 4 * WH),
                 uc, uk, uq(0, qta, 0, 2 * AS), uq(2 * AS, qto, 0, 2 * (US - AS))]
        works = [uw(qto, AS, US - AS), yw(qt2, 0, 2 * YH), ww(qt1, 0, 2 * WH), uw(qta, 0, AS)]
        cc, kc, qc = (4 * CPB, 0, 8 * CPB), (LC[5], 150, 300), (LC[6], 150, 300)
        sched, starts = _plan(preps, pr, works, SPAN3, PROF3, [cc, kc, qc, cc, kc, qc, cc, kc, qc, qc], load)
        assert pr[2] >= pr[1] and starts[1] > max(pr[3], pr[5]) + 200, starts
        assert pr[8] >= pr[7] and starts[2] > max(pr[9], pr[11]) + 200, starts
        assert pr[14] >= pr[13] and min(pr[14], pr[18]) > starts[1] and starts[3] > max(pr[15], pr[17]) + 200, starts
        for h, t in pv_times.items():
            if h < X0:
                assert starts[1] + 400 < t < starts[3], (h, t, starts)
            elif h >= W0:
                assert t > starts[3] + 400, (h, t, starts)
            elif h >= Y0:
                assert t > starts[2] + 400, (h, t, starts)
        r_starts = [t for t, job in jobs if job.func in (o_round, q_round)]

        def in_round(s):
            t = max(t for t in r_starts if t <= s)
            return min(s, t + M - 16)
        holds = [(in_round(starts[1] + HOLD1), LAG1)]
        holds += [(max(t for t in r_starts if t <= s), LAG) for s in (starts[2], starts[3], pr[19] + LAG + M)]
        for t0, job in jobs:
            _emit(sched, t0, job(t0), tokens)
        assert not sched
        return carry

    def body(z, carry):
        carry_buf[0] = jnp.zeros((M, D), F32)
        stage1(z == 77)
        wait_group(len(SEGS))
        lax.fori_loop(0, 2, stage2, 0)
        lax.fori_loop(0, NI, stage3, 0)
        for blk in range(2):
            for n in range(D // DH):
                for r0, rows in out_chunks(n):
                    out_copy(blk, n, r0, rows).wait()
        return carry

    cnt[0] = 1
    lax.fori_loop(0, cnt[0], body, 0)


@jax.jit
def pallas_concat_heads__mha_block_cached__mha_block_cached__near_ridge_kernel(
    A_x: jax.Array,
    A_k_cache: jax.Array,
    A_v_cache: jax.Array,
    A_wq: jax.Array,
    A_wo: jax.Array,
    B_x: jax.Array,
    B_k_cache: jax.Array,
    B_v_cache: jax.Array,
    B_wq: jax.Array,
    B_wo: jax.Array,
):
    def rec16(nh):
        return (nh * B * P16 + 24, 128)

    def rec32(nh):
        return (nh * B * P32 + 40, 128)

    k_t = pltpu.VMEM((DH * P32 + 40, 128), F32)
    out = pl.pallas_call(
        _kernel,
        in_specs=[pl.BlockSpec(memory_space=pl.ANY)] * 10,
        out_specs=pl.BlockSpec(memory_space=pl.ANY),
        out_shape=jax.ShapeDtypeStruct((M, 2 * D), BF16),
        scratch_shapes=[
            pltpu.VMEM((2, M, D), BF16),
            pltpu.VMEM((2, M // 2, D), U32),
            pltpu.VMEM((NI, D, IW + W_PAD), BF16),
            pltpu.VMEM((NI + 1, B, UH, SK, DH), BF16),
            pltpu.VMEM((NI, B, XH, SK, DH), BF16),
            pltpu.VMEM((NI, B, IH - M0, SK, DH), BF16),
            pltpu.VMEM((NI, B, IH, SK, DH), BF16),
            pltpu.VMEM((NI, IW, D + W_PAD), BF16),
            pltpu.VMEM((NI, M, len(MHEADS) * DH), BF16),
            pltpu.VMEM((M // 2, IW), U32),
            pltpu.VMEM((M, 2 * PW), F32),
            pltpu.VMEM((M, D), F32),
            pltpu.VMEM((2, M, D), F32),
            pltpu.VMEM((2, M, D), BF16),
            pltpu.VMEM(rec32(UH), F32),
            pltpu.VMEM((NI - 1,) + rec32(UH), F32),
            pltpu.VMEM((2, XH) + rec32(1), F32),
            pltpu.VMEM((2, XH) + rec32(1), F32),
            pltpu.VMEM((NI,) + rec32(YH), F32),
            pltpu.VMEM(rec32(WH), F32),
            pltpu.VMEM(rec16(UH), U32),
            pltpu.VMEM((NI, XH) + rec16(1), U32),
            pltpu.VMEM(rec16(YH), U32),
            pltpu.VMEM(rec16(WH), U32),
            pltpu.VMEM((SK, 128), F32),
            pltpu.VMEM((len(MHEADS), B // GB, 128, 128), BF16),
            pltpu.VMEM(rec16(UH), U32), k_t,
            pltpu.VMEM((2 * AS, DH, 128), F32),
            pltpu.VMEM((2 * (US - AS), DH, 128), F32),
            pltpu.VMEM(rec16(WH), U32), k_t,
            pltpu.VMEM((4 * WH, DH, 128), F32),
            pltpu.VMEM(rec16(YH), U32), k_t,
            pltpu.VMEM((4 * YH, DH, 128), F32),
            pltpu.SemaphoreType.DMA((NUM_SEMS,)),
            pltpu.SMEM((1,), jnp.int32),
        ],
        compiler_params=pltpu.CompilerParams(
            vmem_limit_bytes=112 * 1024 * 1024,
            disable_bounds_checks=True,
            disable_semaphore_checks=True,
        ),
    )(A_x.reshape(M, D), A_k_cache, A_v_cache, A_wq, A_wo,
      B_x.reshape(M, D), B_k_cache, B_v_cache, B_wq, B_wo)
    return out.reshape(B, SQ, 2 * D)
```
